```python
import os as _os
_os.environ.setdefault("JAX_PLATFORMS", "cpu")
import jax
import jax.numpy as jnp

def _softmax(x, axis=-1):
    return jax.nn.softmax(x, axis=axis)
def _gelu(x):
    return jax.nn.gelu(x, approximate=True)
def _silu(x):
    return jax.nn.silu(x)
def _sigmoid(x):
    return jax.nn.sigmoid(x)
def _layernorm(x, axis=-1, eps=1e-5):
    m = jnp.mean(x, axis=axis, keepdims=True)
    v = jnp.var(x, axis=axis, keepdims=True)
    return (x - m) / jnp.sqrt(v + eps)
def _scatter_add(tgt, idx, src, axis=0):
    return tgt.at[idx].add(src)
def _segment_sum(src, seg, n):
    return jax.ops.segment_sum(src, seg, n)
class _Rng:
    def __init__(self, key):
        self._k = key
    def _next(self):
        self._k, sub = jax.random.split(self._k)
        return sub
    def normal(self, shape):
        return jax.random.normal(self._next(), shape, dtype=jnp.bfloat16)
    def randint(self, lo, hi, shape):
        return jax.random.randint(self._next(), shape, lo, hi, dtype=jnp.int32)
    def uniform(self, shape, lo=0.0, hi=1.0):
        return jax.random.uniform(self._next(), shape, jnp.bfloat16, lo, hi)
    def permutation(self, n):
        return jax.random.permutation(self._next(), n)


kernel_name = 'parallel_sum__mha_block__swiglu_ffn__prompt'

def setup_inputs():
    _rng = _Rng(jax.random.key(int.from_bytes(__import__("os").urandom(4), "little")))
    _w = (lambda a: (lambda t: t.astype(jnp.bfloat16) if jnp.issubdtype(t.dtype, jnp.floating) else t)(jnp.asarray(a)))
    def _A_setup():
        B, S, D, H = 1, 2048, 512, 32
        return {
            "x": _w((lambda *s: _rng.normal(s) * 0.05)(B, S, D)),
            "wqkv": _w((lambda *s: _rng.normal(s) * 0.1)(D, 3 * D)),
            "wo": _w((lambda *s: _rng.normal(s) * 0.05)(D, D)),
        }
    _A_in = _A_setup()

    def _B_setup():
        B, S, D, F = 1, 2048, 512, 1792
        return {
            "x": _w((lambda *s: _rng.normal(s) * 0.05)(B, S, D)),
            "w_gate": _w((lambda *s: _rng.normal(s) * 0.05)(D, F)),
            "w_up": _w((lambda *s: _rng.normal(s) * 0.05)(D, F)),
            "w_down": _w((lambda *s: _rng.normal(s) * 0.05)(F, D)),
        }
    _B_in = _B_setup()

    return {
        "A_x": _A_in["x"],
        "A_wqkv": _A_in["wqkv"],
        "A_wo": _A_in["wo"],
        "B_x": _B_in["x"],
        "B_w_gate": _B_in["w_gate"],
        "B_w_up": _B_in["w_up"],
        "B_w_down": _B_in["w_down"],
    }

def reference(A_x, A_wqkv, A_wo, B_x, B_w_gate, B_w_up, B_w_down):
    def _A_ref(x, wqkv, wo):
        B, S, D = x.shape
        H = 32
        Dh = D // H
        qkv = (lambda x, *d: x.transpose(*d))((x @ wqkv).reshape(B, S, 3, H, Dh), 2, 0, 3, 1, 4)
        q, k, v = qkv[0], qkv[1], qkv[2]
        scores = jnp.einsum("bhqd,bhkd->bhqk", q, k) * (Dh ** -0.5)
        p = _softmax(scores, axis=-1)
        o = jnp.einsum("bhqk,bhkd->bhqd", p, v)
        return (lambda x, *d: x.transpose(*d))(o, 0, 2, 1, 3).reshape(B, S, D) @ wo

    def _B_ref(x, w_gate, w_up, w_down):
        g = _silu(x @ w_gate)
        u = x @ w_up
        return (g * u) @ w_down

    x = A_x
    xn = _layernorm(x, axis=-1)
    return x + _A_ref(xn, A_wqkv, A_wo) + _B_ref(xn, B_w_gate, B_w_up, B_w_down)
```

```python
import jax
import jax.numpy as jnp
import jax.experimental.pallas as pl
import jax.experimental.pallas.tpu as pltpu

H = 32
TQ = 512
KC = 256
PB = 256
LOG2E = 1.4426950408889634
EPS = 1e-5


def _kernel(x_ref, wqkv_ref, wo_ref, wg_ref, wu_ref, wd_ref, o_ref,
            xn_scr, k_scr, qt_scr, vt_scr, s0_scr, s1_scr, ot_scr):
    S, D = x_ref.shape
    Dh = D // H
    HPS = 128 // Dh
    i = pl.program_id(0)
    f32, bf16 = jnp.float32, jnp.bfloat16

    @pl.when(i == 0)
    def _prologue():
        for r in range(S // PB):
            rows = slice(r * PB, (r + 1) * PB)
            x = x_ref[rows, :].astype(f32)
            mu = jnp.mean(x, axis=-1, keepdims=True)
            xc = x - mu
            var = jnp.mean(xc * xc, axis=-1, keepdims=True)
            xn = (xc * jax.lax.rsqrt(var + EPS)).astype(bf16)
            xn_scr[rows, :] = xn
            q = jnp.dot(xn, wqkv_ref[:, 0:D], preferred_element_type=f32)
            qt = (q * (LOG2E * Dh ** -0.5)).T.astype(bf16)
            t, c = (r * PB) // TQ, (r * PB) % TQ
            qt_scr[t, :, c:c + PB] = qt
            k = jnp.dot(xn, wqkv_ref[:, D:2 * D], preferred_element_type=f32).astype(bf16)
            for j in range(D // 128):
                k_scr[j, rows, :] = k[:, j * 128:(j + 1) * 128]
            v = jnp.dot(xn, wqkv_ref[:, 2 * D:3 * D], preferred_element_type=f32)
            vt_scr[:, rows] = v.T.astype(bf16)

    row_head = jax.lax.broadcasted_iota(jnp.int32, (128, TQ), 0) // Dh

    def masked_q(h):
        slab = h // HPS
        qs = qt_scr[i, pl.ds(pl.multiple_of(slab * 128, 128), 128), :]
        return slab, jnp.where(row_head == (h % HPS), qs, jnp.zeros_like(qs))

    def pass1_chunk(slab, qm, s_scr, j, m):
        rows = slice(j * KC, (j + 1) * KC)
        s = jnp.dot(k_scr[slab, rows, :], qm, preferred_element_type=f32)
        s_scr[rows, :] = s
        cm = jnp.max(s.reshape(KC // 8, 8, TQ), axis=0)
        return cm if m is None else jnp.maximum(m, cm)

    def pass2_chunk(h, s_scr, j, m, l, acc):
        rows = slice(j * KC, (j + 1) * KC)
        p = jnp.exp2(s_scr[rows, :].reshape(KC // 8, 8, TQ) - m[None])
        cl = jnp.sum(p, axis=0)
        vt = vt_scr[pl.ds(pl.multiple_of(h * Dh, Dh), Dh), rows]
        pv = jnp.dot(vt, p.reshape(KC, TQ).astype(bf16), preferred_element_type=f32)
        if l is None:
            return cl, pv
        return l + cl, acc + pv

    def fin_max(m):
        return jnp.broadcast_to(jnp.max(m, axis=0, keepdims=True), (8, TQ))

    def step(h1, s_w, h2, s_r, m2):
        m1 = l = acc = None
        if h1 is not None:
            slab, qm = masked_q(h1)
        for j in range(S // KC):
            if h1 is not None:
                m1 = pass1_chunk(slab, qm, s_w, j, m1)
            if h2 is not None:
                l, acc = pass2_chunk(h2, s_r, j, m2, l, acc)
        if h2 is not None:
            inv = 1.0 / jnp.sum(l, axis=0, keepdims=True)
            ot_scr[pl.ds(pl.multiple_of(h2 * Dh, Dh), Dh), :] = (acc * inv).astype(bf16)
        return fin_max(m1) if h1 is not None else None

    m = step(0, s0_scr, None, None, None)

    def pair(t, m):
        h = 2 * t
        m = step(h + 1, s1_scr, h, s0_scr, m)
        m = step(h + 2, s0_scr, h + 1, s1_scr, m)
        return m

    m = jax.lax.fori_loop(0, H // 2 - 1, pair, m)
    m = step(H - 1, s1_scr, H - 2, s0_scr, m)
    step(None, None, H - 1, s1_scr, m)

    rows = pl.ds(pl.multiple_of(i * TQ, TQ), TQ)
    xn = xn_scr[rows, :]
    g = jnp.dot(xn, wg_ref[...], preferred_element_type=f32)
    u = jnp.dot(xn, wu_ref[...], preferred_element_type=f32)
    hmid = (g * jax.nn.sigmoid(g) * u).astype(bf16)
    ffn = jnp.dot(hmid, wd_ref[...], preferred_element_type=f32)
    attn = jax.lax.dot_general(ot_scr[...], wo_ref[...], (((0,), (0,)), ((), ())),
                               preferred_element_type=f32)
    o_ref[...] = (x_ref[rows, :].astype(f32) + attn + ffn).astype(o_ref.dtype)


@jax.jit
def pallas_parallel_sum__mha_block__swiglu_ffn__prompt_kernel(
    A_x, A_wqkv, A_wo, B_x, B_w_gate, B_w_up, B_w_down,
):
    B, S, D = A_x.shape
    F = B_w_gate.shape[1]
    bf16, f32 = jnp.bfloat16, jnp.float32
    x = A_x.reshape(S, D)
    full = lambda a: pl.BlockSpec(a.shape, lambda i: (0,) * a.ndim)
    out = pl.pallas_call(
        _kernel,
        grid=(S // TQ,),
        in_specs=[full(x), full(A_wqkv), full(A_wo), full(B_w_gate), full(B_w_up), full(B_w_down)],
        out_specs=pl.BlockSpec((TQ, D), lambda i: (i, 0)),
        out_shape=jax.ShapeDtypeStruct((S, D), A_x.dtype),
        scratch_shapes=[
            pltpu.VMEM((S, D), bf16),
            pltpu.VMEM((D // 128, S, 128), bf16),
            pltpu.VMEM((S // TQ, D, TQ), bf16),
            pltpu.VMEM((D, S), bf16),
            pltpu.VMEM((S, TQ), f32),
            pltpu.VMEM((S, TQ), f32),
            pltpu.VMEM((D, TQ), bf16),
        ],
        compiler_params=pltpu.CompilerParams(
            dimension_semantics=("arbitrary",),
            vmem_limit_bytes=100 * 1024 * 1024,
        ),
    )(x, A_wqkv, A_wo, B_w_gate, B_w_up, B_w_down)
    return out.reshape(B, S, D)
```

```python
import jax
import jax.numpy as jnp
import jax.experimental.pallas as pl
import jax.experimental.pallas.tpu as pltpu

H = 32
TQ = 512
KC = 128
FC = 128
PB = 256
LOG2E = 1.4426950408889634
EPS = 1e-5


def _kernel(x_hbm, wqkv_hbm, wo_hbm, wg_hbm, wu_hbm, wd_hbm, o_ref,
            x_ref, wqkv_ref, wo_ref, wg_ref, wu_ref, wd_ref, sems,
            xn_scr, k_scr, qt_scr, vt_scr, s_scr, q_scr, ot_scr, m_scr, h_scr):
    S, D = x_ref.shape
    Dh = D // H
    HPS = 128 // Dh
    NB = S // PB
    i = pl.program_id(0)
    f32, bf16 = jnp.float32, jnp.bfloat16

    @pl.when(i == 0)
    def _prologue():
        x_first = pltpu.make_async_copy(x_hbm.at[:2 * PB], x_ref.at[:2 * PB], sems.at[0])
        x_rest = pltpu.make_async_copy(x_hbm.at[2 * PB:], x_ref.at[2 * PB:], sems.at[1])
        wqkv_cp = pltpu.make_async_copy(wqkv_hbm, wqkv_ref, sems.at[2])
        late = [pltpu.make_async_copy(src, dst, sems.at[3 + n]) for n, (src, dst) in enumerate(
            [(wg_hbm, wg_ref), (wu_hbm, wu_ref), (wd_hbm, wd_ref), (wo_hbm, wo_ref)])]
        x_first.start()
        wqkv_cp.start()
        x_first.wait()
        wqkv_cp.wait()
        x_rest.start()
        for r in range(NB):
            if r == 2:
                x_rest.wait()
                for c in late:
                    c.start()
            rows = slice(r * PB, (r + 1) * PB)
            x = x_ref[rows, :].astype(f32)
            mu = jnp.mean(x, axis=-1, keepdims=True)
            xc = x - mu
            var = jnp.mean(xc * xc, axis=-1, keepdims=True)
            xn = (xc * jax.lax.rsqrt(var + EPS)).astype(bf16)
            xn_scr[rows, :] = xn
            q = jnp.dot(xn, wqkv_ref[:, 0:D], preferred_element_type=f32)
            qt = (q * (LOG2E * Dh ** -0.5)).T.astype(bf16)
            t, c = (r * PB) // TQ, (r * PB) % TQ
            qt_scr[t, :, c:c + PB] = qt
            k = jnp.dot(xn, wqkv_ref[:, D:2 * D], preferred_element_type=f32).astype(bf16)
            for j in range(D // 128):
                k_scr[j, rows, :] = k[:, j * 128:(j + 1) * 128]
            v = jnp.dot(xn, wqkv_ref[:, 2 * D:3 * D], preferred_element_type=f32)
            vt_scr[:, rows] = v.T.astype(bf16)
        for c in late:
            c.wait()

    row_head = jax.lax.broadcasted_iota(jnp.int32, (128, TQ), 0) // Dh

    def stage_q(h):
        qs = qt_scr[i, pl.ds(pl.multiple_of((h // HPS) * 128, 128), 128), :]
        q_scr[...] = jnp.where(row_head == (h % HPS), qs, jnp.zeros_like(qs))

    def step(h1, h2, hn, filler=None):
        m1 = l = acc = None
        ls = []
        if h2 is not None:
            m2 = jnp.broadcast_to(jnp.max(m_scr[...], axis=0, keepdims=True), (8, TQ))
            vrows = pl.ds(pl.multiple_of(h2 * Dh, Dh), Dh)
        for j in range(S // KC):
            rows = slice(j * KC, (j + 1) * KC)
            if h2 is not None:
                if j >= 2:
                    m2 = m2 + 0.0 * ls[j - 2]
                p = jnp.exp2(s_scr[rows, :].reshape(KC // 8, 8, TQ) - m2[None])
                cl = jnp.sum(p, axis=0)
                pv = jnp.dot(vt_scr[vrows, rows], p.reshape(KC, TQ).astype(bf16),
                             preferred_element_type=f32)
                l, acc = (cl, pv) if l is None else (l + cl, acc + pv)
                ls.append(l)
            if h1 is not None:
                s = jnp.dot(k_scr[h1 // HPS, rows, :], q_scr[...], preferred_element_type=f32)
                s_scr[rows, :] = s
                cm = jnp.max(s.reshape(KC // 8, 8, TQ), axis=0)
                m1 = cm if m1 is None else jnp.maximum(m1, cm)
            if filler is not None:
                filler(j)
        if hn is not None:
            stage_q(hn)
        if h2 is not None:
            inv = 1.0 / jnp.sum(l, axis=0, keepdims=True)
            ot_scr[vrows, :] = (acc * inv).astype(bf16)
        if h1 is not None:
            m_scr[...] = m1

    stage_q(0)
    step(0, None, 1)

    def body(h, c):
        step(h + 1, h, h + 2)
        return c

    jax.lax.fori_loop(0, H - 2, body, 0)
    step(H - 1, H - 2, None)
    rows = pl.ds(pl.multiple_of(i * TQ, TQ), TQ)
    F = wg_ref.shape[1]

    def gate_up(j):
        c = (j // 1) * FC
        if j % 1 == 0 and c < F:
            xn = xn_scr[rows, :]
            g = jnp.dot(xn, wg_ref[:, c:c + FC], preferred_element_type=f32)
            u = jnp.dot(xn, wu_ref[:, c:c + FC], preferred_element_type=f32)
            h_scr[:, c:c + FC] = (g * jax.nn.sigmoid(g) * u).astype(bf16)

    step(None, H - 1, None, gate_up)
    ffn = jnp.dot(h_scr[...], wd_ref[...], preferred_element_type=f32)
    attn = jax.lax.dot_general(ot_scr[...], wo_ref[...], (((0,), (0,)), ((), ())),
                               preferred_element_type=f32)
    o_ref[...] = (x_ref[rows, :].astype(f32) + attn + ffn).astype(o_ref.dtype)


@jax.jit
def pallas_parallel_sum__mha_block__swiglu_ffn__prompt_kernel(
    A_x, A_wqkv, A_wo, B_x, B_w_gate, B_w_up, B_w_down,
):
    B, S, D = A_x.shape
    bf16, f32 = jnp.bfloat16, jnp.float32
    x = A_x.reshape(S, D)
    ins = (x, A_wqkv, A_wo, B_w_gate, B_w_up, B_w_down)
    out = pl.pallas_call(
        _kernel,
        grid=(S // TQ,),
        in_specs=[pl.BlockSpec(memory_space=pl.ANY)] * len(ins),
        out_specs=pl.BlockSpec((TQ, D), lambda i: (i, 0)),
        out_shape=jax.ShapeDtypeStruct((S, D), A_x.dtype),
        scratch_shapes=[pltpu.VMEM(a.shape, a.dtype) for a in ins] + [
            pltpu.SemaphoreType.DMA((7,)),
            pltpu.VMEM((S, D), bf16),
            pltpu.VMEM((D // 128, S, 128), bf16),
            pltpu.VMEM((S // TQ, D, TQ), bf16),
            pltpu.VMEM((D, S), bf16),
            pltpu.VMEM((S, TQ), f32),
            pltpu.VMEM((128, TQ), bf16),
            pltpu.VMEM((D, TQ), bf16),
            pltpu.VMEM((8, TQ), f32),
            pltpu.VMEM((TQ, B_w_gate.shape[1]), bf16),
        ],
        compiler_params=pltpu.CompilerParams(
            dimension_semantics=("arbitrary",),
            vmem_limit_bytes=100 * 1024 * 1024,
        ),
    )(*ins)
    return out.reshape(B, S, D)
```
